```python
import jax
import jax.numpy as jnp

def _softmax(x, axis=-1):
    return jax.nn.softmax(x, axis=axis)

def _gelu(x):
    return jax.nn.gelu(x, approximate=True)

def _silu(x):
    return jax.nn.silu(x)

def _sigmoid(x):
    return jax.nn.sigmoid(x)

def _layernorm(x, axis=-1, eps=1e-05):
    m = jnp.mean(x, axis=axis, keepdims=True)
    v = jnp.var(x, axis=axis, keepdims=True)
    return (x - m) / jnp.sqrt(v + eps)

def _scatter_add(tgt, idx, src, axis=0):
    return tgt.at[idx].add(src)

def _segment_sum(src, seg, n):
    return jax.ops.segment_sum(src, seg, n)

class _Rng:

    def __init__(self, key):
        self._k = key

    def _next(self):
        self._k, sub = jax.random.split(self._k)
        return sub

    def normal(self, shape):
        return jax.random.normal(self._next(), shape, dtype=jnp.bfloat16)

    def randint(self, lo, hi, shape):
        return jax.random.randint(self._next(), shape, lo, hi, dtype=jnp.int32)

    def uniform(self, shape, lo=0.0, hi=1.0):
        return jax.random.uniform(self._next(), shape, jnp.bfloat16, lo, hi)

    def permutation(self, n):
        return jax.random.permutation(self._next(), n)
kernel_name = 'standalone__window_attn_davit__vision'

def setup_inputs():
    _rng = _Rng(jax.random.key(int.from_bytes(__import__("os").urandom(4), "little")))
    _w = lambda a: (lambda t: t.astype(jnp.bfloat16) if jnp.issubdtype(t.dtype, jnp.floating) else t)(jnp.asarray(a))
    HW = 512
    C0 = 192
    ws = 7
    nh = 4
    H = W = max(HW // ws * ws, ws)
    C = max(C0 // nh * nh, nh)
    k = 3
    return {'x': _w((lambda *s: _rng.normal(s) * 0.05)(1, H, W, C)), 'dw_pe': _w((lambda *s: _rng.normal(s) * 0.05)(k, k, C) * 0.1), 'w_qkv': _w((lambda *s: _rng.normal(s) * 0.05)(C, 3 * C) * C ** (-0.5)), 'w_o': _w((lambda *s: _rng.normal(s) * 0.05)(C, C) * C ** (-0.5))}

def reference(x, dw_pe, w_qkv, w_o):
    B, H, W, C = x.shape
    ws = 7
    nh = 4
    dh = C // nh
    kk = dw_pe.shape[0]
    pad = kk // 2
    xp = jnp.pad(x, ((0, 0), (pad, pad), (pad, pad), (0, 0)))
    pe = jnp.zeros_like(x)
    for i in range(kk):
        for j in range(kk):
            pe = pe + xp[:, i:i + H, j:j + W, :] * dw_pe[i, j][None, None, None, :]
    x0 = x + pe
    h = _layernorm(x0, axis=-1)
    hw = h.reshape(B, H // ws, ws, W // ws, ws, C)
    hw = (lambda x, *d: x.transpose(*d))(hw, 0, 1, 3, 2, 4, 5)
    hw = hw.reshape(-1, ws * ws, C)
    qkv = (hw @ w_qkv).reshape(-1, ws * ws, 3, nh, dh)
    q = qkv[:, :, 0].copy()
    k = qkv[:, :, 1].copy()
    v = qkv[:, :, 2].copy()
    scale = dh ** (-0.5)
    attn = jnp.einsum('wnhd,wmhd->whnm', q, k) * scale
    attn = _softmax(attn, axis=-1)
    out = jnp.einsum('whnm,wmhd->wnhd', attn, v)
    out = out.reshape(-1, ws * ws, C) @ w_o
    out = out.reshape(B, H // ws, W // ws, ws, ws, C)
    out = (lambda x, *d: x.transpose(*d))(out, 0, 1, 3, 2, 4, 5)
    out = out.reshape(B, H, W, C)
    return x0 + out
```

```python
import functools
import math

import jax
import jax.numpy as jnp
from jax import lax
import jax.experimental.pallas as pl
import jax.experimental.pallas.tpu as pltpu

F32 = jnp.float32
BF16 = jnp.bfloat16

WS = 7
NH = 4
C = 192
DH = C // NH
HH = 511
WP = 512
NWIN = HH // WS
RING = 16
MODE = __import__('os').environ.get('MODE', 'sw')
DEPTH = int(__import__('os').environ.get('DEPTH', 2))
UNROLL = int(__import__('os').environ.get('UNR', 4))


def _nt(a, b):
    return lax.dot_general(a, b, (((1,), (1,)), ((), ())), preferred_element_type=F32)


def _nn(a, b):
    return lax.dot_general(a, b, (((1,), (0,)), ((), ())), preferred_element_type=F32)


def _tn(a, b):
    return lax.dot_general(a, b, (((0,), (0,)), ((), ())), preferred_element_type=F32)


def _sub_reduce(x, op):
    x = op(x, pltpu.roll(x, 4, 0))
    x = op(x, pltpu.roll(x, 2, 0))
    x = op(x, pltpu.roll(x, 1, 0))
    return x


def _kernel(xm_ref, xn_ref, dw_ref, wqkv_ref, wo_ref, o_ref,
            xs, x0s, hts, qkv, os_, w640, woT):
    s = pl.program_id(0)
    nsteps = pl.num_programs(0)

    lane = lax.broadcasted_iota(jnp.int32, (1, 128), 1)

    @pl.when(s == 0)
    def _prep():
        wq = wqkv_ref[:, 0:C].astype(F32) * (DH ** -0.5 * math.log2(math.e))
        wq = wq.astype(BF16)
        wk = wqkv_ref[:, C:2 * C]
        wv = wqkv_ref[:, 2 * C:3 * C]
        z32 = jnp.zeros((C, 32), BF16)
        v13 = jnp.concatenate([wv[:, DH:2 * DH], wv[:, 3 * DH:4 * DH]], axis=1)
        t0 = jnp.concatenate([v13[:, 0:32], wq[:, 0:96]], axis=1)
        t1 = jnp.concatenate([z32, wk[:, 0:96]], axis=1)
        t2 = jnp.concatenate([wq[:, 96:128], v13[:, 32:64], wq[:, 128:192]], axis=1)
        t3 = jnp.concatenate([wk[:, 96:128], z32, wk[:, 128:192]], axis=1)
        t4 = jnp.concatenate([wv[:, 0:DH], wv[:, 2 * DH:3 * DH], v13[:, 64:96]], axis=1)
        w640[:, 0:128] = t0
        w640[:, 128:256] = t1
        w640[:, 256:384] = t2
        w640[:, 384:512] = t3
        w640[:, 512:640] = t4
        wo = wo_ref[...]
        zr = jnp.zeros((32, C), BF16)
        r02 = jnp.concatenate([wo[0:DH], wo[2 * DH:3 * DH], zr], axis=0)
        r13 = jnp.concatenate([wo[DH:2 * DH], wo[3 * DH:3 * DH + 16], zr,
                               wo[3 * DH + 16:4 * DH]], axis=0)
        woT[0] = r02.astype(F32).T.astype(BF16)
        woT[1] = r13.astype(F32).T.astype(BF16)
        xs[RING - 1] = jnp.zeros((C, WP), F32)
        for t in range(2):
            os_[t, pl.ds(0, 8), :] = jnp.zeros((8, 128), F32)

    wmask = lax.broadcasted_iota(jnp.int32, (1, WP), 1) < HH

    def put_row(slot, src, valid=None):
        v = src.astype(F32)
        m = wmask if valid is None else jnp.logical_and(wmask, valid)
        xs[slot] = jnp.where(m, v, 0.0)

    @pl.when(s == 0)
    def _():
        put_row(0, xm_ref[0])

    def load_body(k, c):
        put_row((WS * s + k) % RING, xm_ref[k])
        return c
    lax.fori_loop(1, WS, load_body, 0)
    put_row((WS * s + WS) % RING, xn_ref[0], s < nsteps - 1)

    def row_body(r, c):
        g = WS * s + r
        sl_t = (g + RING - 1) % RING
        sl_m = g % RING
        sl_b = (g + 1) % RING
        CH = 16
        ssum = jnp.zeros((8, WP), F32)
        for ci in range(C // CH):
            rows = pl.ds(ci * CH, CH)
            top = xs[sl_t, rows, :]
            mid = xs[sl_m, rows, :]
            bot = xs[sl_b, rows, :]

            def coef(i, j):
                cf = dw_ref[i * 3 + j, rows, :]
                return jnp.concatenate([cf] * (WP // 128), axis=1)

            t0 = top * coef(0, 0) + mid * coef(1, 0) + bot * coef(2, 0)
            t1 = top * coef(0, 1) + mid * coef(1, 1) + bot * coef(2, 1)
            t2 = top * coef(0, 2) + mid * coef(1, 2) + bot * coef(2, 2)
            t0s = pltpu.roll(t0, 1, 1)
            t2s = pltpu.roll(t2, WP - 1, 1)
            x0 = mid + (t0s + t1 + t2s)
            x0s[r, rows, :] = x0
            ssum = ssum + (x0[0:8] + x0[8:16])
        mean = _sub_reduce(ssum, jnp.add) * (1.0 / C)
        mean2 = jnp.concatenate([mean, mean], axis=0)
        vsum = jnp.zeros((8, WP), F32)
        for ci in range(C // CH):
            rows = pl.ds(ci * CH, CH)
            d = x0s[r, rows, :] - mean2
            dd = d * d
            vsum = vsum + (dd[0:8] + dd[8:16])
        var = _sub_reduce(vsum, jnp.add) * (1.0 / C)
        rstd = lax.rsqrt(var + 1e-5)
        rstd2 = jnp.concatenate([rstd, rstd], axis=0)
        for ci in range(C // CH):
            rows = pl.ds(ci * CH, CH)
            d = x0s[r, rows, :] - mean2
            hts[rows, :] = (d * rstd2).astype(BF16)

        base = pl.multiple_of(r * WP, WP)
        TCH = 256
        for tc in range(WP // TCH):
            ht = hts[:, tc * TCH:(tc + 1) * TCH]
            res = _tn(ht, w640[...])
            trow = pl.ds(base + tc * TCH, TCH)
            t0 = res[:, 0:128]
            t2 = res[:, 256:384]
            t4 = res[:, 512:640]
            qkv[0, trow, :] = t0
            qkv[1, trow, :] = res[:, 128:256]
            qkv[2, trow, :] = t2
            qkv[3, trow, :] = res[:, 384:512]
            qkv[4, trow, :] = t4
            qkv[5, trow, :] = jnp.where(lane < 32, t0, jnp.where(lane < 64, t2, t4))
        return c

    lax.fori_loop(0, WS, row_body, 0)

    sub = lax.broadcasted_iota(jnp.int32, (8, 128), 0)
    key_ok = sub < WS
    ln = lax.broadcasted_iota(jnp.int32, (8, 128), 1)
    mq = [
        jnp.logical_and(ln >= 32, ln < 80),
        ln >= 80,
        jnp.logical_or(ln < 32, jnp.logical_and(ln >= 64, ln < 80)),
        ln >= 80,
    ]
    mv = [
        ln < 48,
        jnp.logical_and(ln >= 48, ln < 96),
        jnp.logical_or(jnp.logical_and(ln >= 48, ln < 64), ln >= 96),
    ]
    zero8 = jnp.zeros((8, 128), F32)

    def load56(t, off):
        return [qkv[t, pl.ds(off + WP * rr, 8), :] for rr in range(WS)]

    def pack64(parts):
        return jnp.concatenate(parts + [zero8], axis=0).astype(BF16)

    def bd(parts, ma, mb):
        za = [jnp.where(ma, v, 0.0) for v in parts] + [zero8]
        zb = [jnp.where(mb, v, 0.0) for v in parts] + [zero8]
        return jnp.concatenate(za + zb, axis=0).astype(BF16)

    def softmax_t(st):
        parts = [st[8 * i:8 * i + 8] for i in range(WS)]
        m = parts[0]
        for p in parts[1:]:
            m = jnp.maximum(m, p)
        m = jnp.where(key_ok, m, -jnp.inf)
        m = _sub_reduce(m, jnp.maximum)
        m = jnp.where(key_ok, m, jnp.inf)
        es = [jnp.exp2(p - m) for p in parts]
        l = es[0]
        for e in es[1:]:
            l = l + e
        l = _sub_reduce(l, jnp.add)
        rcp = pl.reciprocal(l, approx=True)
        rcp = rcp * (2.0 - l * rcp)
        return pack64([e * rcp for e in es])

    def ph_qk(j):
        off = WS * j
        k01 = jnp.concatenate(load56(1, off), axis=0)
        k23 = jnp.concatenate(load56(3, off), axis=0)
        q01 = bd(load56(0, off), mq[0], mq[1])
        q23 = bd(load56(2, off), mq[2], mq[3])
        return _nt(k01, q01), _nt(k23, q23)

    def ph_sm(ss):
        z = jnp.concatenate([softmax_t(ss[0]), softmax_t(ss[1])], axis=0)
        return z.T

    def ph_pv(j, zt):
        off = WS * j
        v02 = bd(load56(4, off), mv[0], mv[1])
        v13 = bd(load56(5, off), mv[0], mv[2])
        o02 = _nn(zt[0:64], v02)
        o13 = _nn(zt[64:128], v13)
        for rr in range(WS):
            os_[0, pl.ds(off + WP * rr, 8), :] = o02[8 * rr:8 * rr + 8]
            os_[1, pl.ds(off + WP * rr, 8), :] = o13[8 * rr:8 * rr + 8]

    def windows(js):
        ss = [ph_qk(j) for j in js]
        zs = [ph_sm(x) for x in ss]
        for j, z in zip(js, zs):
            ph_pv(j, z)

    if MODE == "loop":
        UNR = UNROLL

        def win_body(i, c):
            windows([i * UNR + u for u in range(UNR)])
            return c
        lax.fori_loop(0, NWIN // UNR, win_body, 0)
        windows(list(range(NWIN // UNR * UNR, NWIN)))
    else:
        D = DEPTH
        ss, zs = {}, {}
        for t in range(NWIN + 2 * D):
            if t < NWIN:
                ss[t] = ph_qk(t)
            if 0 <= t - D < NWIN:
                zs[t - D] = ph_sm(ss.pop(t - D))
            if 0 <= t - 2 * D < NWIN:
                ph_pv(t - 2 * D, zs.pop(t - 2 * D))

    def out_body(r, c):
        base = pl.multiple_of(r * WP, WP)
        o02 = os_[0, pl.ds(base, WP), :].astype(BF16)
        o13 = os_[1, pl.ds(base, WP), :].astype(BF16)
        acc = _nt(woT[0], o02) + _nt(woT[1], o13)
        o_ref[r] = (x0s[r] + acc).astype(BF16)
        return c
    lax.fori_loop(0, WS, out_body, 0)


@jax.jit
def pallas_standalone__window_attn_davit__vision_kernel(
    x: jax.Array,
    dw_pe: jax.Array,
    w_qkv: jax.Array,
    w_o: jax.Array,
):
    B, H, W, Cc = x.shape
    xt = x.reshape(H, W, Cc).transpose(0, 2, 1)
    dwb = jnp.broadcast_to(dw_pe.reshape(9, Cc, 1), (9, Cc, 128)).astype(F32)

    out = pl.pallas_call(
        _kernel,
        grid=(NWIN,),
        in_specs=[
            pl.BlockSpec((WS, Cc, WP), lambda s: (s, 0, 0)),
            pl.BlockSpec((1, Cc, WP), lambda s: (jnp.minimum(WS * s + WS, H - 1), 0, 0)),
            pl.BlockSpec((9, Cc, 128), lambda s: (0, 0, 0)),
            pl.BlockSpec((Cc, 3 * Cc), lambda s: (0, 0)),
            pl.BlockSpec((Cc, Cc), lambda s: (0, 0)),
        ],
        out_specs=pl.BlockSpec((WS, Cc, WP), lambda s: (s, 0, 0)),
        out_shape=jax.ShapeDtypeStruct((H, Cc, W), x.dtype),
        scratch_shapes=[
            pltpu.VMEM((RING, Cc, WP), F32),
            pltpu.VMEM((WS, Cc, WP), F32),
            pltpu.VMEM((Cc, WP), BF16),
            pltpu.VMEM((6, WS * WP + 8, 128), F32),
            pltpu.VMEM((2, WS * WP + 8, 128), F32),
            pltpu.VMEM((Cc, 640), BF16),
            pltpu.VMEM((2, Cc, 128), BF16),
        ],
        compiler_params=pltpu.CompilerParams(
            dimension_semantics=("arbitrary",),
            vmem_limit_bytes=100 * 1024 * 1024,
        ),
    )(xt, xt, dwb, w_qkv, w_o)
    return out.transpose(0, 2, 1).reshape(B, H, W, Cc)
```

```python
import functools
import math

import jax
import jax.numpy as jnp
from jax import lax
import jax.experimental.pallas as pl
import jax.experimental.pallas.tpu as pltpu

F32 = jnp.float32
BF16 = jnp.bfloat16

WS = 7
NH = 4
C = 192
DH = C // NH
HH = 511
WP = 512
NWIN = HH // WS
RING = 14
_env = __import__('os').environ
TCH = int(_env.get('TCH', 128))
ZCH = int(_env.get('ZCH', 128))
INFLIGHT = int(_env.get('INFLIGHT', 6))
LAG_QK = int(_env.get('LAG_QK', 120))
LAG_TR = int(_env.get('LAG_TR', 100))
VALU_AHEAD = float(_env.get('VALU_AHEAD', 1.1))
VALU_SLACK = float(_env.get('VALU_SLACK', 50))


def _nt(a, b):
    return lax.dot_general(a, b, (((1,), (1,)), ((), ())), preferred_element_type=F32)


def _nn(a, b):
    return lax.dot_general(a, b, (((1,), (0,)), ((), ())), preferred_element_type=F32)


def _tn(a, b):
    return lax.dot_general(a, b, (((0,), (0,)), ((), ())), preferred_element_type=F32)


def _sub_reduce(x, op):
    x = op(x, pltpu.roll(x, 4, 0))
    x = op(x, pltpu.roll(x, 2, 0))
    x = op(x, pltpu.roll(x, 1, 0))
    return x


def _kernel(xm_ref, xn_ref, dw_ref, wqkv_ref, wo_ref, o_ref,
            xs, x0s, hts, qkv, os_, w640, woT):
    s = pl.program_id(0)
    nsteps = pl.num_programs(0)

    lane = lax.broadcasted_iota(jnp.int32, (1, 128), 1)

    @pl.when(s == 0)
    def _prep():
        wq = wqkv_ref[:, 0:C].astype(F32) * (DH ** -0.5 * math.log2(math.e))
        wq = wq.astype(BF16)
        wk = wqkv_ref[:, C:2 * C]
        wv = wqkv_ref[:, 2 * C:3 * C]
        z32 = jnp.zeros((C, 32), BF16)
        v13 = jnp.concatenate([wv[:, DH:2 * DH], wv[:, 3 * DH:4 * DH]], axis=1)
        t0 = jnp.concatenate([v13[:, 0:32], wq[:, 0:96]], axis=1)
        t1 = jnp.concatenate([z32, wk[:, 0:96]], axis=1)
        t2 = jnp.concatenate([wq[:, 96:128], v13[:, 32:64], wq[:, 128:192]], axis=1)
        t3 = jnp.concatenate([wk[:, 96:128], z32, wk[:, 128:192]], axis=1)
        t4 = jnp.concatenate([wv[:, 0:DH], wv[:, 2 * DH:3 * DH], v13[:, 64:96]], axis=1)
        w640[:, 0:128] = t0
        w640[:, 128:256] = t1
        w640[:, 256:384] = t2
        w640[:, 384:512] = t3
        w640[:, 512:640] = t4
        wo = wo_ref[...]
        zr = jnp.zeros((32, C), BF16)
        r02 = jnp.concatenate([wo[0:DH], wo[2 * DH:3 * DH], zr], axis=0)
        r13 = jnp.concatenate([wo[DH:2 * DH], wo[3 * DH:3 * DH + 16], zr,
                               wo[3 * DH + 16:4 * DH]], axis=0)
        woT[0] = r02.astype(F32).T.astype(BF16)
        woT[1] = r13.astype(F32).T.astype(BF16)
        xs[RING - 1] = jnp.zeros((C, WP), F32)
        hts[WS - 1] = jnp.zeros((C, WP), BF16)
        x0s[1] = jnp.zeros((WS, C, WP), F32)

        def zbody(i, c):
            rows = pl.ds(pl.multiple_of(i * 8, 8), 8)
            for t in range(6):
                qkv[1, t, rows, :] = jnp.zeros((8, 128), F32)
            return c
        lax.fori_loop(0, WS * WP // 8 + 1, zbody, 0)
        for t in range(6):
            qkv[0, t, pl.ds(WS * WP, 8), :] = jnp.zeros((8, 128), F32)

    wmask = lax.broadcasted_iota(jnp.int32, (1, WP), 1) < HH
    last = nsteps - 2

    def put_rows(slot, rows, src, valid=None):
        v = src.astype(F32)
        m = wmask if valid is None else jnp.logical_and(wmask, valid)
        xs[slot, rows, :] = jnp.where(m, v, 0.0)

    @pl.when(s == 0)
    def _():
        put_rows(0, pl.ds(0, C), xm_ref[0])

    def step(cur):
        prv = 1 - cur
        g0 = WS * cur
        tasks = []

        def add(name, fn, deps=(), mxu=0, valu=0, prio=0):
            tasks.append(dict(name=name, fn=fn, deps=list(deps), mxu=mxu, valu=valu, prio=prio))

        UCH = 48
        for k in range(1, WS + 1):
            for ui in range(C // UCH):
                def f(k=k, ui=ui):
                    rows = pl.ds(ui * UCH, UCH)
                    if k < WS:
                        put_rows((g0 + k) % RING, rows, xm_ref[k, rows, :])
                    else:
                        put_rows((g0 + k) % RING, rows, xn_ref[0, rows, :], s < last)
                add(("U", k, ui), f, valu=28, prio=(k - 1) * 100 + ui)

        st = {}
        CH = 8
        NCI = C // CH
        for r in range(WS):
            for ci in range(NCI):
                def f(r=r, ci=ci):
                    rows = pl.ds(ci * CH, CH)
                    top = xs[(g0 + r + RING - 1) % RING, rows, :]
                    mid = xs[(g0 + r) % RING, rows, :]
                    bot = xs[(g0 + r + 1) % RING, rows, :]

                    def coef(i, j):
                        cf = dw_ref[i * 3 + j, rows, :]
                        return jnp.concatenate([cf] * (WP // 128), axis=1)

                    t0 = top * coef(0, 0) + mid * coef(1, 0) + bot * coef(2, 0)
                    t1 = top * coef(0, 1) + mid * coef(1, 1) + bot * coef(2, 1)
                    t2 = top * coef(0, 2) + mid * coef(1, 2) + bot * coef(2, 2)
                    x0 = mid + (pltpu.roll(t0, 1, 1) + t1 + pltpu.roll(t2, WP - 1, 1))
                    x0s[cur, r, rows, :] = x0
                    st[("s", r)] = x0 if ci == 0 else st[("s", r)] + x0
                deps = [(("U", r + 1, ci * CH // UCH), 40)]
                if ci:
                    deps.append((("C", r, ci - 1), 0))
                add(("C", r, ci), f, deps, valu=24, prio=r * 100 + 10 + ci)

            def f(r=r):
                st[("m", r)] = _sub_reduce(st.pop(("s", r)), jnp.add) * (1.0 / C)
            add(("M", r), f, [(("C", r, NCI - 1), 0)], valu=8, prio=r * 100 + 40)

            for ci in range(C // 16):
                def f(r=r, ci=ci):
                    mean = st[("m", r)]
                    acc = None
                    for hf in range(2):
                        d = x0s[cur, r, pl.ds(ci * 16 + hf * 8, 8), :] - mean
                        acc = d * d if acc is None else acc + d * d
                    st[("v", r)] = acc if ci == 0 else st[("v", r)] + acc
                deps = [(("M", r), 10)] if ci == 0 else [(("V", r, ci - 1), 0)]
                add(("V", r, ci), f, deps, valu=6, prio=r * 100 + 50 + ci)

            def f(r=r):
                var = _sub_reduce(st.pop(("v", r)), jnp.add) * (1.0 / C)
                st[("r", r)] = lax.rsqrt(var + 1e-5)
            add(("R", r), f, [(("V", r, C // 16 - 1), 0)], valu=10, prio=r * 100 + 70)

            for ci in range(C // 16):
                def f(r=r, ci=ci):
                    mean = st[("m", r)]
                    rstd = st[("r", r)]
                    rows = pl.ds(ci * 16, 16)
                    d = x0s[cur, r, rows, :] - jnp.concatenate([mean, mean], axis=0)
                    hts[r, rows, :] = (d * jnp.concatenate([rstd, rstd], axis=0)).astype(BF16)
                deps = [(("R", r), 30)]
                if r == WS - 1:
                    deps.append((("Q", -1, WP // TCH - 1), 0))
                add(("N", r, ci), f, deps, valu=6, prio=r * 100 + 80 + ci)

        for r in range(-1, WS - 1):
            for tc in range(WP // TCH):
                def f(r=r, tc=tc):
                    rr = r % WS
                    slot = prv if r < 0 else cur
                    ht = hts[rr, :, tc * TCH:(tc + 1) * TCH]
                    res = _tn(ht, w640[...])
                    trow = pl.ds(rr * WP + tc * TCH, TCH)
                    t0 = res[:, 0:128]
                    t2 = res[:, 256:384]
                    t4 = res[:, 512:640]
                    qkv[slot, 0, trow, :] = t0
                    qkv[slot, 1, trow, :] = res[:, 128:256]
                    qkv[slot, 2, trow, :] = t2
                    qkv[slot, 3, trow, :] = res[:, 384:512]
                    qkv[slot, 4, trow, :] = t4
                    qkv[slot, 5, trow, :] = jnp.where(lane < 32, t0, jnp.where(lane < 64, t2, t4))
                deps = []
                if r >= 0:
                    deps.append((("N", r, C // 16 - 1), 60))
                if tc:
                    deps.append((("Q", r, tc - 1), 0))
                elif r >= 0:
                    deps.append((("Q", r - 1, WP // TCH - 1), 0))
                add(("Q", r, tc), f, deps, mxu=TCH * 10 // 4, valu=TCH * 112 // 128 // 4, prio=2)

        sub = lax.broadcasted_iota(jnp.int32, (8, 128), 0)
        key_ok = sub < WS
        ln = lax.broadcasted_iota(jnp.int32, (8, 128), 1)
        mq = [
            jnp.logical_and(ln >= 32, ln < 80),
            ln >= 80,
            jnp.logical_or(ln < 32, jnp.logical_and(ln >= 64, ln < 80)),
            ln >= 80,
        ]
        mv = [
            ln < 48,
            jnp.logical_and(ln >= 48, ln < 96),
            jnp.logical_or(jnp.logical_and(ln >= 48, ln < 64), ln >= 96),
        ]
        zero8 = jnp.zeros((8, 128), F32)

        def load56(t, off):
            return [qkv[prv, t, pl.ds(off + WP * rr, 8), :] for rr in range(WS)]

        def pack64(parts):
            return jnp.concatenate(parts + [zero8], axis=0).astype(BF16)

        def bd(parts, ma, mb):
            za = [jnp.where(ma, v, 0.0) for v in parts] + [zero8]
            zb = [jnp.where(mb, v, 0.0) for v in parts] + [zero8]
            return jnp.concatenate(za + zb, axis=0).astype(BF16)

        def softmax_t(stv):
            parts = [stv[8 * i:8 * i + 8] for i in range(WS)]
            m = parts[0]
            for p in parts[1:]:
                m = jnp.maximum(m, p)
            m = jnp.where(key_ok, m, -jnp.inf)
            m = _sub_reduce(m, jnp.maximum)
            m = jnp.where(key_ok, m, jnp.inf)
            es = [jnp.exp2(p - m) for p in parts]
            l = es[0]
            for e in es[1:]:
                l = l + e
            l = _sub_reduce(l, jnp.add)
            rcp = pl.reciprocal(l, approx=True)
            rcp = rcp * (2.0 - l * rcp)
            return pack64([e * rcp for e in es])

        for w in range(NWIN):
            off = WS * w
            tcw = min((off + 7) // TCH, WP // TCH - 1)

            def f_qk(w=w, off=off):
                k01 = jnp.concatenate(load56(1, off), axis=0)
                k23 = jnp.concatenate(load56(3, off), axis=0)
                q01 = bd(load56(0, off), mq[0], mq[1])
                q23 = bd(load56(2, off), mq[2], mq[3])
                st[("S", w)] = (_nt(k01, q01), _nt(k23, q23))
            deps = [(("Q", -1, tcw), 200)]
            if w:
                deps.append((("QK", w - 1), 0))
            if w >= INFLIGHT:
                deps.append((("PV", w - INFLIGHT), 0))
            add(("QK", w), f_qk, deps, mxu=28, valu=5, prio=1)

            for hp in range(2):
                def f_sm(w=w, hp=hp):
                    st[("P", w, hp)] = softmax_t(st[("S", w)][hp])
                    if hp == 1:
                        del st[("S", w)]
                add(("SM", w, hp), f_sm, [(("QK", w), LAG_QK)] + ([(("SM", w, 0), 0)] if hp else []),
                    valu=14, prio=-1)

            def f_tr(w=w):
                z = jnp.concatenate([st.pop(("P", w, 0)), st.pop(("P", w, 1))], axis=0)
                st[("Z", w)] = z.T
            add(("TR", w), f_tr, [(("SM", w, 1), 20)], valu=6, prio=-2)

            def f_pv(w=w, off=off):
                zt = st.pop(("Z", w))
                v02 = bd(load56(4, off), mv[0], mv[1])
                v13 = bd(load56(5, off), mv[0], mv[2])
                o02 = _nn(zt[0:64], v02)
                o13 = _nn(zt[64:128], v13)
                for rr in range(WS):
                    os_[0, pl.ds(off + WP * rr, 8), :] = o02[8 * rr:8 * rr + 8]
                    os_[1, pl.ds(off + WP * rr, 8), :] = o13[8 * rr:8 * rr + 8]
            deps = [(("TR", w), LAG_TR)]
            if w:
                deps.append((("PV", w - 1), 0))
            add(("PV", w), f_pv, deps, mxu=32, valu=3, prio=0)

        for tc in range(WP // ZCH):
            wlast = min((tc * ZCH + ZCH - 1) // WS, NWIN - 1)
            for r in range(WS):
                def f(r=r, tc=tc):
                    trow = pl.ds(r * WP + tc * ZCH, ZCH)
                    o02 = os_[0, trow, :].astype(BF16)
                    o13 = os_[1, trow, :].astype(BF16)
                    acc = _nt(woT[0], o02) + _nt(woT[1], o13)
                    cols = pl.ds(tc * ZCH, ZCH)
                    o_ref[r, :, cols] = (x0s[prv, r, :, cols] + acc).astype(BF16)
                add(("Z", r, tc), f, [(("PV", wlast), 150)], mxu=ZCH * 3 // 4, valu=ZCH * 21 // 128, prio=3)

        _emit(tasks)

    for par in range(2):
        pl.when(s % 2 == par)(functools.partial(step, par))


def _emit(tasks):
    tot_mxu = sum(t["mxu"] for t in tasks)
    tot_valu = sum(t["valu"] for t in tasks)
    ratio = tot_valu / tot_mxu * VALU_AHEAD
    done = {}
    pending = list(tasks)
    now = 0.0
    cum_valu = 0.0
    while pending:
        ready, soonest = [], None
        for t in pending:
            if all(d in done for d, _ in t["deps"]):
                t_ok = max([done[d] + lag for d, lag in t["deps"]], default=0.0)
                if t_ok <= now:
                    ready.append(t)
                else:
                    soonest = t_ok if soonest is None else min(soonest, t_ok)
        if not ready:
            now = soonest
            continue
        mx = [t for t in ready if t["mxu"]]
        va = [t for t in ready if not t["mxu"]]
        pick = None
        if va:
            v = min(va, key=lambda t: t["prio"])
            if not mx or v["prio"] < 0 or cum_valu < ratio * now + VALU_SLACK:
                pick = v
        if pick is None:
            pick = min(mx, key=lambda t: t["prio"])
        pending.remove(pick)
        pick["fn"]()
        now += pick["mxu"]
        cum_valu += pick["valu"]
        if not pick["mxu"] and not mx:
            now += pick["valu"]
        done[pick["name"]] = now


@jax.jit
def pallas_standalone__window_attn_davit__vision_kernel(
    x: jax.Array,
    dw_pe: jax.Array,
    w_qkv: jax.Array,
    w_o: jax.Array,
):
    B, H, W, Cc = x.shape
    xt = x.reshape(H, W, Cc).transpose(0, 2, 1)
    dwb = jnp.broadcast_to(dw_pe.reshape(9, Cc, 1), (9, Cc, 128)).astype(F32)

    out = pl.pallas_call(
        _kernel,
        grid=(NWIN + 1,),
        in_specs=[
            pl.BlockSpec((WS, Cc, WP), lambda s: (jnp.minimum(s, NWIN - 1), 0, 0)),
            pl.BlockSpec((1, Cc, WP), lambda s: (jnp.minimum(WS * s + WS, H - 1), 0, 0)),
            pl.BlockSpec((9, Cc, 128), lambda s: (0, 0, 0)),
            pl.BlockSpec((Cc, 3 * Cc), lambda s: (0, 0)),
            pl.BlockSpec((Cc, Cc), lambda s: (0, 0)),
        ],
        out_specs=pl.BlockSpec((WS, Cc, WP), lambda s: (jnp.maximum(s - 1, 0), 0, 0)),
        out_shape=jax.ShapeDtypeStruct((H, Cc, W), x.dtype),
        scratch_shapes=[
            pltpu.VMEM((RING, Cc, WP), F32),
            pltpu.VMEM((2, WS, Cc, WP), F32),
            pltpu.VMEM((WS, Cc, WP), BF16),
            pltpu.VMEM((2, 6, WS * WP + 8, 128), F32),
            pltpu.VMEM((2, WS * WP + 8, 128), F32),
            pltpu.VMEM((Cc, 640), BF16),
            pltpu.VMEM((2, Cc, 128), BF16),
        ],
        compiler_params=pltpu.CompilerParams(
            dimension_semantics=("arbitrary",),
            vmem_limit_bytes=100 * 1024 * 1024,
        ),
    )(xt, xt, dwb, w_qkv, w_o)
    return out.transpose(0, 2, 1).reshape(B, H, W, Cc)
```

```python
import functools
import math

import jax
import jax.numpy as jnp
from jax import lax
import jax.experimental.pallas as pl
import jax.experimental.pallas.tpu as pltpu

F32 = jnp.float32
BF16 = jnp.bfloat16
U32 = jnp.uint32

WS = 7
NH = 4
C = 192
DH = C // NH
HH = 511
WP = 512
NWIN = HH // WS
RING = 14
TCH = 128
ZCH = 128
INFLIGHT = 8
LAG_QK = 120
LAG_TR = 100
ATT_BEG = 500.0
ATT_END = 0.85
Q_SHIFT = 0.0
U_AHEAD = 0.3
C_OFF = -0.1
C_LEN = 0.6
V_EARLY = 0.0
NS = 16
STAGE_S = 1
STAGE_Z = 1
TR_LAG = 60
KFLAGS = ''


def _nt(a, b):
    return lax.dot_general(a, b, (((1,), (1,)), ((), ())), preferred_element_type=F32)


def _nn(a, b):
    return lax.dot_general(a, b, (((1,), (0,)), ((), ())), preferred_element_type=F32)


def _tn(a, b):
    return lax.dot_general(a, b, (((0,), (0,)), ((), ())), preferred_element_type=F32)


def _sub_reduce(x, op):
    x = op(x, pltpu.roll(x, 4, 0))
    x = op(x, pltpu.roll(x, 2, 0))
    x = op(x, pltpu.roll(x, 1, 0))
    return x


def _kernel(xm_ref, xn_ref, dw_ref, wqkv_ref, wo_ref, o_ref,
            xs, x0s, hts, qkv, os_, w640, woT, s_scr, z_scr):
    s = pl.program_id(0)
    nsteps = pl.num_programs(0)

    lane = lax.broadcasted_iota(jnp.int32, (1, 128), 1)

    @pl.when(s == 0)
    def _prep():
        wq = wqkv_ref[:, 0:C].astype(F32) * (DH ** -0.5 * math.log2(math.e))
        wq = wq.astype(BF16)
        wk = wqkv_ref[:, C:2 * C]
        wv = wqkv_ref[:, 2 * C:3 * C]
        z32 = jnp.zeros((C, 32), BF16)
        v13 = jnp.concatenate([wv[:, DH:2 * DH], wv[:, 3 * DH:4 * DH]], axis=1)
        t0 = jnp.concatenate([v13[:, 0:32], wq[:, 0:96]], axis=1)
        t1 = jnp.concatenate([z32, wk[:, 0:96]], axis=1)
        t2 = jnp.concatenate([wq[:, 96:128], v13[:, 32:64], wq[:, 128:192]], axis=1)
        t3 = jnp.concatenate([wk[:, 96:128], z32, wk[:, 128:192]], axis=1)
        t4 = jnp.concatenate([wv[:, 0:DH], wv[:, 2 * DH:3 * DH], v13[:, 64:96]], axis=1)
        w640[:, 0:128] = pltpu.bitcast(t0, U32)
        w640[:, 128:256] = pltpu.bitcast(t1, U32)
        w640[:, 256:384] = pltpu.bitcast(t2, U32)
        w640[:, 384:512] = pltpu.bitcast(t3, U32)
        w640[:, 512:640] = pltpu.bitcast(t4, U32)
        wo = wo_ref[...]
        zr = jnp.zeros((32, C), BF16)
        r02 = jnp.concatenate([wo[0:DH], wo[2 * DH:3 * DH], zr], axis=0)
        r13 = jnp.concatenate([wo[DH:2 * DH], wo[3 * DH:3 * DH + 16], zr,
                               wo[3 * DH + 16:4 * DH]], axis=0)
        woT[0] = pltpu.bitcast(r02.astype(F32).T.astype(BF16), U32)
        woT[1] = pltpu.bitcast(r13.astype(F32).T.astype(BF16), U32)
        xs[RING - 1] = jnp.zeros((C, WP), F32)
        hts[WS - 1] = jnp.zeros((C // 2, WP), U32)
        x0s[1] = jnp.zeros((WS, C, WP), F32)

        def zbody(i, c):
            rows = pl.ds(pl.multiple_of(i * 8, 8), 8)
            for t in range(6):
                qkv[1, t, rows, :] = jnp.zeros((8, 128), F32)
            return c
        lax.fori_loop(0, WS * WP // 8 + 1, zbody, 0)
        for t in range(6):
            qkv[0, t, pl.ds(WS * WP, 8), :] = jnp.zeros((8, 128), F32)

    wmask = lax.broadcasted_iota(jnp.int32, (1, WP), 1) < HH
    last = nsteps - 2

    def put_rows(slot, rows, src, valid=None):
        v = src.astype(F32)
        m = wmask if valid is None else jnp.logical_and(wmask, valid)
        xs[slot, rows, :] = jnp.where(m, v, 0.0)

    @pl.when(s == 0)
    def _():
        put_rows(0, pl.ds(0, C), xm_ref[0])

    def step(cur):
        prv = 1 - cur
        g0 = WS * cur
        tasks = []

        def add(name, fn, deps=(), mxu=0, valu=0, prio=0):
            tasks.append(dict(name=name, fn=fn, deps=list(deps), mxu=mxu, valu=valu, prio=prio))

        UCH = 48
        for k in range(1, WS + 1):
            for ui in range(C // UCH):
                def f(k=k, ui=ui):
                    rows = pl.ds(ui * UCH, UCH)
                    if k < WS:
                        put_rows((g0 + k) % RING, rows, xm_ref[k, rows, :])
                    else:
                        put_rows((g0 + k) % RING, rows, xn_ref[0, rows, :], s < last)
                add(("U", k, ui), f, valu=28, prio=(k - 1) * 100 + ui)

        st = {}
        CH = 8
        NCI = C // CH
        for r in range(WS):
            for ci in range(NCI):
                def f(r=r, ci=ci):
                    rows = pl.ds(ci * CH, CH)
                    top = xs[(g0 + r + RING - 1) % RING, rows, :]
                    mid = xs[(g0 + r) % RING, rows, :]
                    bot = xs[(g0 + r + 1) % RING, rows, :]

                    def coef(i, j):
                        cf = dw_ref[i * 3 + j, rows, :]
                        return jnp.concatenate([cf] * (WP // 128), axis=1)

                    t0 = top * coef(0, 0) + mid * coef(1, 0) + bot * coef(2, 0)
                    t1 = top * coef(0, 1) + mid * coef(1, 1) + bot * coef(2, 1)
                    t2 = top * coef(0, 2) + mid * coef(1, 2) + bot * coef(2, 2)
                    x0 = mid + (pltpu.roll(t0, 1, 1) + t1 + pltpu.roll(t2, WP - 1, 1))
                    x0s[cur, r, rows, :] = x0
                    st[("s", r)] = x0 if ci == 0 else st[("s", r)] + x0
                deps = [(("U", r + 1, ci * CH // UCH), 40)]
                if ci:
                    deps.append((("C", r, ci - 1), 0))
                add(("C", r, ci), f, deps, valu=24, prio=r * 100 + 10 + ci)

            def f(r=r):
                st[("m", r)] = _sub_reduce(st.pop(("s", r)), jnp.add) * (1.0 / C)
            add(("M", r), f, [(("C", r, NCI - 1), 0)], valu=8, prio=r * 100 + 40)

            for ci in range(C // 16):
                def f(r=r, ci=ci):
                    mean = st[("m", r)]
                    acc = None
                    for hf in range(2):
                        d = x0s[cur, r, pl.ds(ci * 16 + hf * 8, 8), :] - mean
                        acc = d * d if acc is None else acc + d * d
                    st[("v", r)] = acc if ci == 0 else st[("v", r)] + acc
                deps = [(("M", r), 10)] if ci == 0 else [(("V", r, ci - 1), 0)]
                add(("V", r, ci), f, deps, valu=6, prio=r * 100 + 50 + ci)

            def f(r=r):
                var = _sub_reduce(st.pop(("v", r)), jnp.add) * (1.0 / C)
                st[("r", r)] = lax.rsqrt(var + 1e-5)
                st[("o", r)] = -st[("m", r)] * st[("r", r)]
            add(("R", r), f, [(("V", r, C // 16 - 1), 0)], valu=10, prio=r * 100 + 70)

            for ci in range(C // 16):
                def f(r=r, ci=ci):
                    rstd = st[("r", r)]
                    rows = pl.ds(ci * 16, 16)
                    shift = st[("o", r)]
                    hv = (x0s[cur, r, rows, :] * jnp.concatenate([rstd, rstd], axis=0)
                          + jnp.concatenate([shift, shift], axis=0)).astype(BF16)
                    hts[r, pl.ds(ci * 8, 8), :] = pltpu.bitcast(hv, U32)
                deps = [(("R", r), 30)]
                if r == WS - 1:
                    deps.append((("Q", -1, WP // TCH - 1), 0))
                add(("N", r, ci), f, deps, valu=6, prio=r * 100 + 80 + ci)

        for r in range(-1, WS - 1):
            for tc in range(WP // TCH):
                def f(r=r, tc=tc):
                    rr = r % WS
                    slot = prv if r < 0 else cur
                    ht = pltpu.bitcast(hts[rr, :, tc * TCH:(tc + 1) * TCH], BF16)
                    res = _tn(ht, pltpu.bitcast(w640[...], BF16))
                    trow = pl.ds(rr * WP + tc * TCH, TCH)
                    t0 = res[:, 0:128]
                    t2 = res[:, 256:384]
                    t4 = res[:, 512:640]
                    qkv[slot, 0, trow, :] = t0
                    qkv[slot, 1, trow, :] = res[:, 128:256]
                    qkv[slot, 2, trow, :] = t2
                    qkv[slot, 3, trow, :] = res[:, 384:512]
                    qkv[slot, 4, trow, :] = t4
                    qkv[slot, 5, trow, :] = jnp.where(lane < 32, t0, jnp.where(lane < 64, t2, t4))
                deps = []
                if r >= 0:
                    deps.append((("N", r, C // 16 - 1), 60))
                if tc:
                    deps.append((("Q", r, tc - 1), 0))
                elif r >= 0:
                    deps.append((("Q", r - 1, WP // TCH - 1), 0))
                add(("Q", r, tc), f, deps, mxu=TCH * 10 // 4, valu=TCH * 112 // 128 // 4, prio=2)

        sub = lax.broadcasted_iota(jnp.int32, (8, 128), 0)
        key_ok = sub < WS
        ln = lax.broadcasted_iota(jnp.int32, (8, 128), 1)
        mq = [
            jnp.logical_and(ln >= 32, ln < 80),
            ln >= 80,
            jnp.logical_or(ln < 32, jnp.logical_and(ln >= 64, ln < 80)),
            ln >= 80,
        ]
        mv = [
            ln < 48,
            jnp.logical_and(ln >= 48, ln < 96),
            jnp.logical_or(jnp.logical_and(ln >= 48, ln < 64), ln >= 96),
        ]
        zero8 = jnp.zeros((8, 128), F32)

        def load56(t, off):
            return [qkv[prv, t, pl.ds(off + WP * rr, 8), :] for rr in range(WS)]

        def pack64(parts):
            return jnp.concatenate(parts + [zero8], axis=0).astype(BF16)

        def bd(parts, ma, mb):
            za = [jnp.where(ma, v, 0.0) for v in parts] + [zero8]
            zb = [jnp.where(mb, v, 0.0) for v in parts] + [zero8]
            return jnp.concatenate(za + zb, axis=0).astype(BF16)

        def softmax_t(stv):
            parts = [stv[8 * i:8 * i + 8] for i in range(WS)]
            m = parts[0]
            for p in parts[1:]:
                m = jnp.maximum(m, p)
            m = jnp.where(key_ok, m, -jnp.inf)
            m = _sub_reduce(m, jnp.maximum)
            m = jnp.where(key_ok, m, jnp.inf)
            es = [jnp.exp2(p - m) for p in parts]
            l = es[0]
            for e in es[1:]:
                l = l + e
            l = _sub_reduce(l, jnp.add)
            rcp = pl.reciprocal(l, approx=True)
            rcp = rcp * (2.0 - l * rcp)
            return pack64([e * rcp for e in es])

        for w in range(NWIN):
            off = WS * w
            tcw = min((off + 7) // TCH, WP // TCH - 1)

            def f_qk(w=w, off=off):
                k01 = jnp.concatenate(load56(1, off), axis=0)
                k23 = jnp.concatenate(load56(3, off), axis=0)
                q01 = bd(load56(0, off), mq[0], mq[1])
                q23 = bd(load56(2, off), mq[2], mq[3])
                if STAGE_S:
                    s_scr[w % NS, 0] = _nt(k01, q01)
                    s_scr[w % NS, 1] = _nt(k23, q23)
                else:
                    st[("S", w)] = (_nt(k01, q01), _nt(k23, q23))
            deps = [(("Q", -1, tcw), 200)]
            if w:
                deps.append((("QK", w - 1), 0))
            if w >= INFLIGHT:
                deps.append((("PV", w - INFLIGHT), 0))
            add(("QK", w), f_qk, deps, mxu=28, valu=5, prio=1)

            for hp in range(2):
                def f_sm(w=w, hp=hp):
                    if STAGE_S:
                        st[("P", w, hp)] = softmax_t(s_scr[w % NS, hp])
                    else:
                        st[("P", w, hp)] = softmax_t(st[("S", w)][hp])
                        if hp == 1:
                            del st[("S", w)]
                add(("SM", w, hp), f_sm, [(("QK", w), LAG_QK)] + ([(("SM", w, 0), 0)] if hp else []),
                    valu=14, prio=-1)

            def f_tr(w=w):
                z = jnp.concatenate([st.pop(("P", w, 0)), st.pop(("P", w, 1))], axis=0)
                zt = z.T
                if STAGE_Z:
                    z_scr[w % NS] = pltpu.bitcast(zt, U32)
                else:
                    st[("Z", w)] = (zt[0:64], zt[64:128])
            add(("TR", w), f_tr, [(("SM", w, 1), 20)], valu=6, prio=-2)

            def f_pv(w=w, off=off):
                if STAGE_Z:
                    zt = (pltpu.bitcast(z_scr[w % NS, 0:32], BF16),
                          pltpu.bitcast(z_scr[w % NS, 32:64], BF16))
                else:
                    zt = st.pop(("Z", w))
                v02 = bd(load56(4, off), mv[0], mv[1])
                v13 = bd(load56(5, off), mv[0], mv[2])
                o02 = _nn(zt[0], v02)
                o13 = _nn(zt[1], v13)
                for rr in range(WS):
                    os_[0, pl.ds(off + WP * rr, 8), :] = o02[8 * rr:8 * rr + 8]
                    os_[1, pl.ds(off + WP * rr, 8), :] = o13[8 * rr:8 * rr + 8]
            deps = [(("TR", w), LAG_TR)]
            if w:
                deps.append((("PV", w - 1), 0))
            add(("PV", w), f_pv, deps, mxu=32, valu=3, prio=0)

        for tc in range(WP // ZCH):
            wlast = min((tc * ZCH + ZCH - 1) // WS, NWIN - 1)
            for r in range(WS):
                def f(r=r, tc=tc):
                    trow = pl.ds(r * WP + tc * ZCH, ZCH)
                    o02 = os_[0, trow, :].astype(BF16)
                    o13 = os_[1, trow, :].astype(BF16)
                    acc = (_nt(pltpu.bitcast(woT[0], BF16), o02)
                           + _nt(pltpu.bitcast(woT[1], BF16), o13))
                    cols = pl.ds(tc * ZCH, ZCH)
                    o_ref[r, :, cols] = (x0s[prv, r, :, cols] + acc).astype(BF16)
                add(("Z", r, tc), f, [(("PV", wlast), 150)], mxu=ZCH * 3 // 4, valu=ZCH * 21 // 128, prio=3)

        _emit(tasks)

    for par in range(2):
        pl.when(s % 2 == par)(functools.partial(step, par))


def _emit(tasks):
    T = float(sum(t["mxu"] for t in tasks))
    row = T / WS
    nq = WP // TCH
    qk = lambda w: ATT_BEG + w * (ATT_END * T - ATT_BEG) / NWIN
    pv = lambda w: qk(w) + LAG_QK + TR_LAG + LAG_TR
    zlast = lambda tc: min((tc * ZCH + ZCH - 1) // WS, NWIN - 1)
    for t in tasks:
        n = t["name"]
        k = n[0]
        if k == "Q":
            tau = ((n[1] + 1) * nq + n[2]) * row / nq + Q_SHIFT
        elif k == "U":
            tau = (n[1] - 1) * row - U_AHEAD * row + n[2] * 30
        elif k == "C":
            tau = (n[1] + C_OFF + C_LEN * n[2] / (C // 8)) * row
        elif k == "M":
            tau = (n[1] + C_OFF + C_LEN + 0.01) * row
        elif k == "V":
            tau = (n[1] + C_OFF + C_LEN + 0.02 + 0.08 * n[2] / 12) * row
        elif k == "R":
            tau = (n[1] + C_OFF + C_LEN + 0.11) * row
        elif k == "N":
            tau = (n[1] + C_OFF + C_LEN + 0.13 + 0.1 * n[2] / 12) * row
        elif k == "QK":
            tau = qk(n[1])
        elif k == "SM":
            tau = qk(n[1]) + LAG_QK + n[2]
        elif k == "TR":
            tau = qk(n[1]) + LAG_QK + TR_LAG
        elif k == "PV":
            tau = pv(n[1])
        elif k == "Z":
            beg = pv(zlast(n[2])) + 150
            end = pv(zlast(n[2] + 1)) + 150 if (n[2] + 1) * ZCH < WP else T - 100
            tau = beg + n[1] * (end - beg) / WS
        t["tau"] = tau
    done = {}
    pending = sorted(tasks, key=lambda t: t["tau"])
    now = 0.0
    while pending:
        pick, soonest = None, None
        for t in pending:
            if all(d in done for d, _ in t["deps"]):
                t_ok = max([done[d] + lag for d, lag in t["deps"]], default=0.0)
                if not t["mxu"]:
                    t_ok = max(t_ok, t["tau"] - V_EARLY)
                if t_ok <= now:
                    pick = t
                    break
                soonest = t_ok if soonest is None else min(soonest, t_ok)
        if pick is None:
            now = soonest
            continue
        pending.remove(pick)
        pick["fn"]()
        now += pick["mxu"]
        done[pick["name"]] = now


@jax.jit
def pallas_standalone__window_attn_davit__vision_kernel(
    x: jax.Array,
    dw_pe: jax.Array,
    w_qkv: jax.Array,
    w_o: jax.Array,
):
    B, H, W, Cc = x.shape
    xt = x.reshape(H, W, Cc).transpose(0, 2, 1)
    dwb = jnp.broadcast_to(dw_pe.reshape(9, Cc, 1), (9, Cc, 128)).astype(F32)

    out = pl.pallas_call(
        _kernel,
        grid=(NWIN + 1,),
        in_specs=[
            pl.BlockSpec((WS, Cc, WP), lambda s: (jnp.minimum(s, NWIN - 1), 0, 0)),
            pl.BlockSpec((1, Cc, WP), lambda s: (jnp.minimum(WS * s + WS, H - 1), 0, 0)),
            pl.BlockSpec((9, Cc, 128), lambda s: (0, 0, 0)),
            pl.BlockSpec((Cc, 3 * Cc), lambda s: (0, 0)),
            pl.BlockSpec((Cc, Cc), lambda s: (0, 0)),
        ],
        out_specs=pl.BlockSpec((WS, Cc, WP), lambda s: (jnp.maximum(s - 1, 0), 0, 0)),
        out_shape=jax.ShapeDtypeStruct((H, Cc, W), x.dtype),
        scratch_shapes=[
            pltpu.VMEM((RING, Cc, WP), F32),
            pltpu.VMEM((2, WS, Cc, WP), F32),
            pltpu.VMEM((WS, Cc // 2, WP), U32),
            pltpu.VMEM((2, 6, WS * WP + 8, 128), F32),
            pltpu.VMEM((2, WS * WP + 8, 128), F32),
            pltpu.VMEM((Cc // 2, 640), U32),
            pltpu.VMEM((2, Cc // 2, 128), U32),
            pltpu.VMEM((NS, 2, 56, 128), F32),
            pltpu.VMEM((NS, 64, 128), U32),
        ],
        compiler_params=pltpu.CompilerParams(
            dimension_semantics=("arbitrary",),
            vmem_limit_bytes=100 * 1024 * 1024,
            flags={k: True for k in KFLAGS.split(',') if k} or None,
        ),
    )(xt, xt, dwb, w_qkv, w_o)
    return out.transpose(0, 2, 1).reshape(B, H, W, Cc)
```

```python
import functools
import math

import jax
import jax.numpy as jnp
from jax import lax
import jax.experimental.pallas as pl
import jax.experimental.pallas.tpu as pltpu

F32 = jnp.float32
BF16 = jnp.bfloat16
U32 = jnp.uint32

WS = 7
NH = 4
C = 192
DH = C // NH
HH = 511
WP = 512
NWIN = HH // WS
RING = 14
TCH = 128
ZCH = 128
INFLIGHT = 8
LAG_QK = 120
LAG_TR = 100
ATT_BEG = 500.0
ATT_END = 0.85
Q_SHIFT = 0.0
U_AHEAD = 0.3
C_OFF = -0.1
C_LEN = 0.6
V_EARLY = 0.0
NS = 16
STAGE_S = 1
STAGE_Z = 1
TR_LAG = 60
KFLAGS = ''


def _nt(a, b):
    return lax.dot_general(a, b, (((1,), (1,)), ((), ())), preferred_element_type=F32)


def _nn(a, b):
    return lax.dot_general(a, b, (((1,), (0,)), ((), ())), preferred_element_type=F32)


def _tn(a, b):
    return lax.dot_general(a, b, (((0,), (0,)), ((), ())), preferred_element_type=F32)


def _pack2(lo, hi):
    u = pltpu.pack_elementwise([lo, hi], packed_dtype=BF16)
    return u if u.dtype == U32 else pltpu.bitcast(u, U32)


def _pack_rows(t):
    t = t.astype(F32)
    return jnp.concatenate(
        [_pack2(t[16 * g:16 * g + 8], t[16 * g + 8:16 * g + 16]) for g in range(t.shape[0] // 16)], axis=0)


def _sub_reduce(x, op):
    x = op(x, pltpu.roll(x, 4, 0))
    x = op(x, pltpu.roll(x, 2, 0))
    x = op(x, pltpu.roll(x, 1, 0))
    return x


def _kernel(xm_ref, xn_ref, dw_ref, wqkv_ref, wo_ref, o_ref,
            xs, x0s, hts, qkv, os_, w640, woT, s_scr, z_scr):
    s = pl.program_id(0)
    nsteps = pl.num_programs(0)

    lane = lax.broadcasted_iota(jnp.int32, (1, 128), 1)

    @pl.when(s == 0)
    def _prep():
        wq = wqkv_ref[:, 0:C].astype(F32) * (DH ** -0.5 * math.log2(math.e))
        wq = wq.astype(BF16)
        wk = wqkv_ref[:, C:2 * C]
        wv = wqkv_ref[:, 2 * C:3 * C]
        z32 = jnp.zeros((C, 32), BF16)
        v13 = jnp.concatenate([wv[:, DH:2 * DH], wv[:, 3 * DH:4 * DH]], axis=1)
        t0 = jnp.concatenate([v13[:, 0:32], wq[:, 0:96]], axis=1)
        t1 = jnp.concatenate([z32, wk[:, 0:96]], axis=1)
        t2 = jnp.concatenate([wq[:, 96:128], v13[:, 32:64], wq[:, 128:192]], axis=1)
        t3 = jnp.concatenate([wk[:, 96:128], z32, wk[:, 128:192]], axis=1)
        t4 = jnp.concatenate([wv[:, 0:DH], wv[:, 2 * DH:3 * DH], v13[:, 64:96]], axis=1)
        w640[:, 0:128] = _pack_rows(t0)
        w640[:, 128:256] = _pack_rows(t1)
        w640[:, 256:384] = _pack_rows(t2)
        w640[:, 384:512] = _pack_rows(t3)
        w640[:, 512:640] = _pack_rows(t4)
        wo = wo_ref[...]
        zr = jnp.zeros((32, C), BF16)
        r02 = jnp.concatenate([wo[0:DH], wo[2 * DH:3 * DH], zr], axis=0)
        r13 = jnp.concatenate([wo[DH:2 * DH], wo[3 * DH:3 * DH + 16], zr,
                               wo[3 * DH + 16:4 * DH]], axis=0)
        woT[0] = pltpu.bitcast(r02.astype(F32).T.astype(BF16), U32)
        woT[1] = pltpu.bitcast(r13.astype(F32).T.astype(BF16), U32)
        xs[RING - 1] = jnp.zeros((C, WP), F32)
        hts[WS - 1] = jnp.zeros((C // 2, WP), U32)
        x0s[1] = jnp.zeros((WS, C, WP), F32)

        def zbody(i, c):
            rows = pl.ds(pl.multiple_of(i * 8, 8), 8)
            for t in range(6):
                qkv[1, t, rows, :] = jnp.zeros((8, 128), F32)
            return c
        lax.fori_loop(0, WS * WP // 8 + 1, zbody, 0)
        for t in range(6):
            qkv[0, t, pl.ds(WS * WP, 8), :] = jnp.zeros((8, 128), F32)

    wmask = lax.broadcasted_iota(jnp.int32, (1, WP), 1) < HH
    last = nsteps - 2

    def put_rows(slot, rows, src, valid=None):
        v = src.astype(F32)
        m = wmask if valid is None else jnp.logical_and(wmask, valid)
        xs[slot, rows, :] = jnp.where(m, v, 0.0)

    @pl.when(s == 0)
    def _():
        put_rows(0, pl.ds(0, C), xm_ref[0])

    def step(cur):
        prv = 1 - cur
        g0 = WS * cur
        tasks = []

        def add(name, fn, deps=(), mxu=0, valu=0, prio=0):
            tasks.append(dict(name=name, fn=fn, deps=list(deps), mxu=mxu, valu=valu, prio=prio))

        UCH = 48
        for k in range(1, WS + 1):
            for ui in range(C // UCH):
                def f(k=k, ui=ui):
                    rows = pl.ds(ui * UCH, UCH)
                    if k < WS:
                        put_rows((g0 + k) % RING, rows, xm_ref[k, rows, :])
                    else:
                        put_rows((g0 + k) % RING, rows, xn_ref[0, rows, :], s < last)
                add(("U", k, ui), f, valu=28, prio=(k - 1) * 100 + ui)

        st = {}
        CH = 8
        NCI = C // CH
        for r in range(WS):
            for ci in range(NCI):
                def f(r=r, ci=ci):
                    rows = pl.ds(ci * CH, CH)
                    top = xs[(g0 + r + RING - 1) % RING, rows, :]
                    mid = xs[(g0 + r) % RING, rows, :]
                    bot = xs[(g0 + r + 1) % RING, rows, :]

                    def coef(i, j):
                        cf = dw_ref[i * 3 + j, rows, :]
                        return jnp.concatenate([cf] * (WP // 128), axis=1)

                    t0 = top * coef(0, 0) + mid * coef(1, 0) + bot * coef(2, 0)
                    t1 = top * coef(0, 1) + mid * coef(1, 1) + bot * coef(2, 1)
                    t2 = top * coef(0, 2) + mid * coef(1, 2) + bot * coef(2, 2)
                    x0 = mid + (pltpu.roll(t0, 1, 1) + t1 + pltpu.roll(t2, WP - 1, 1))
                    x0s[cur, r, rows, :] = x0
                    st[("s", r)] = x0 if ci == 0 else st[("s", r)] + x0
                deps = [(("U", r + 1, ci * CH // UCH), 40)]
                if ci:
                    deps.append((("C", r, ci - 1), 0))
                add(("C", r, ci), f, deps, valu=24, prio=r * 100 + 10 + ci)

            def f(r=r):
                st[("m", r)] = _sub_reduce(st.pop(("s", r)), jnp.add) * (1.0 / C)
            add(("M", r), f, [(("C", r, NCI - 1), 0)], valu=8, prio=r * 100 + 40)

            for ci in range(C // 16):
                def f(r=r, ci=ci):
                    mean = st[("m", r)]
                    acc = None
                    for hf in range(2):
                        d = x0s[cur, r, pl.ds(ci * 16 + hf * 8, 8), :] - mean
                        acc = d * d if acc is None else acc + d * d
                    st[("v", r)] = acc if ci == 0 else st[("v", r)] + acc
                deps = [(("M", r), 10)] if ci == 0 else [(("V", r, ci - 1), 0)]
                add(("V", r, ci), f, deps, valu=6, prio=r * 100 + 50 + ci)

            def f(r=r):
                var = _sub_reduce(st.pop(("v", r)), jnp.add) * (1.0 / C)
                st[("r", r)] = lax.rsqrt(var + 1e-5)
                st[("o", r)] = -st[("m", r)] * st[("r", r)]
            add(("R", r), f, [(("V", r, C // 16 - 1), 0)], valu=10, prio=r * 100 + 70)

            for ci in range(C // 16):
                def f(r=r, ci=ci):
                    rstd = st[("r", r)]
                    shift = st[("o", r)]
                    lo = x0s[cur, r, pl.ds(ci * 16, 8), :] * rstd + shift
                    hi = x0s[cur, r, pl.ds(ci * 16 + 8, 8), :] * rstd + shift
                    hts[r, pl.ds(ci * 8, 8), :] = _pack2(lo, hi)
                deps = [(("R", r), 30)]
                if r == WS - 1:
                    deps.append((("Q", -1, WP // TCH - 1), 0))
                add(("N", r, ci), f, deps, valu=6, prio=r * 100 + 80 + ci)

        for r in range(-1, WS - 1):
            for tc in range(WP // TCH):
                def f(r=r, tc=tc):
                    rr = r % WS
                    slot = prv if r < 0 else cur
                    ht = pltpu.bitcast(hts[rr, :, tc * TCH:(tc + 1) * TCH], BF16)
                    res = _tn(ht, pltpu.bitcast(w640[...], BF16))
                    trow = pl.ds(rr * WP + tc * TCH, TCH)
                    t0 = res[:, 0:128]
                    t2 = res[:, 256:384]
                    t4 = res[:, 512:640]
                    qkv[slot, 0, trow, :] = t0
                    qkv[slot, 1, trow, :] = res[:, 128:256]
                    qkv[slot, 2, trow, :] = t2
                    qkv[slot, 3, trow, :] = res[:, 384:512]
                    qkv[slot, 4, trow, :] = t4
                    qkv[slot, 5, trow, :] = jnp.where(lane < 32, t0, jnp.where(lane < 64, t2, t4))
                deps = []
                if r >= 0:
                    deps.append((("N", r, C // 16 - 1), 60))
                if tc:
                    deps.append((("Q", r, tc - 1), 0))
                elif r >= 0:
                    deps.append((("Q", r - 1, WP // TCH - 1), 0))
                add(("Q", r, tc), f, deps, mxu=TCH * 10 // 4, valu=TCH * 112 // 128 // 4, prio=2)

        sub = lax.broadcasted_iota(jnp.int32, (8, 128), 0)
        key_ok = sub < WS
        ln = lax.broadcasted_iota(jnp.int32, (8, 128), 1)
        mq = [
            jnp.logical_and(ln >= 32, ln < 80),
            ln >= 80,
            jnp.logical_or(ln < 32, jnp.logical_and(ln >= 64, ln < 80)),
            ln >= 80,
        ]
        ones = jnp.full((8, 128), 0xFFFFFFFF, U32)
        zeros = jnp.zeros((8, 128), U32)
        mv = [
            jnp.where(ln < 48, ones, zeros),
            jnp.where(jnp.logical_and(ln >= 48, ln < 96), ones, zeros),
            jnp.where(jnp.logical_or(jnp.logical_and(ln >= 48, ln < 64), ln >= 96), ones, zeros),
        ]
        zero8 = jnp.zeros((8, 128), F32)

        def load56(t, off):
            return [qkv[prv, t, pl.ds(off + WP * rr, 8), :] for rr in range(WS)]

        def pack64(parts):
            pz = parts + [zero8]
            return [_pack2(pz[2 * i], pz[2 * i + 1]) for i in range(4)]

        def bd(parts, ma, mb):
            za = [jnp.where(ma, v, 0.0) for v in parts] + [zero8]
            zb = [jnp.where(mb, v, 0.0) for v in parts] + [zero8]
            return jnp.concatenate(za + zb, axis=0).astype(BF16)

        def bdv(parts, ma, mb):
            us = pack64(parts)
            return pltpu.bitcast(jnp.concatenate([u & ma for u in us] + [u & mb for u in us], axis=0), BF16)

        def softmax_t(stv):
            parts = [stv[8 * i:8 * i + 8] for i in range(WS)]
            m = parts[0]
            for p in parts[1:]:
                m = jnp.maximum(m, p)
            m = jnp.where(key_ok, m, -jnp.inf)
            m = _sub_reduce(m, jnp.maximum)
            m = jnp.where(key_ok, m, jnp.inf)
            es = [jnp.exp2(p - m) for p in parts]
            l = es[0]
            for e in es[1:]:
                l = l + e
            l = _sub_reduce(l, jnp.add)
            rcp = pl.reciprocal(l, approx=True)
            rcp = rcp * (2.0 - l * rcp)
            return pack64([e * rcp for e in es])

        for w in range(NWIN):
            off = WS * w
            tcw = min((off + 7) // TCH, WP // TCH - 1)

            def f_qk(w=w, off=off):
                k01 = jnp.concatenate(load56(1, off), axis=0)
                k23 = jnp.concatenate(load56(3, off), axis=0)
                q01 = bd(load56(0, off), mq[0], mq[1])
                q23 = bd(load56(2, off), mq[2], mq[3])
                if STAGE_S:
                    s_scr[w % NS, 0] = _nt(k01, q01)
                    s_scr[w % NS, 1] = _nt(k23, q23)
                else:
                    st[("S", w)] = (_nt(k01, q01), _nt(k23, q23))
            deps = [(("Q", -1, tcw), 200)]
            if w:
                deps.append((("QK", w - 1), 0))
            if w >= INFLIGHT:
                deps.append((("PV", w - INFLIGHT), 0))
            add(("QK", w), f_qk, deps, mxu=28, valu=5, prio=1)

            for hp in range(2):
                def f_sm(w=w, hp=hp):
                    if STAGE_S:
                        st[("P", w, hp)] = softmax_t(s_scr[w % NS, hp])
                    else:
                        st[("P", w, hp)] = softmax_t(st[("S", w)][hp])
                        if hp == 1:
                            del st[("S", w)]
                add(("SM", w, hp), f_sm, [(("QK", w), LAG_QK)] + ([(("SM", w, 0), 0)] if hp else []),
                    valu=14, prio=-1)

            def f_tr(w=w):
                z = pltpu.bitcast(jnp.concatenate(st.pop(("P", w, 0)) + st.pop(("P", w, 1)), axis=0), BF16)
                zt = z.T
                if STAGE_Z:
                    z_scr[w % NS] = pltpu.bitcast(zt, U32)
                else:
                    st[("Z", w)] = (zt[0:64], zt[64:128])
            add(("TR", w), f_tr, [(("SM", w, 1), 20)], valu=6, prio=-2)

            def f_pv(w=w, off=off):
                if STAGE_Z:
                    zt = (pltpu.bitcast(z_scr[w % NS, 0:32], BF16),
                          pltpu.bitcast(z_scr[w % NS, 32:64], BF16))
                else:
                    zt = st.pop(("Z", w))
                v02 = bdv(load56(4, off), mv[0], mv[1])
                v13 = bdv(load56(5, off), mv[0], mv[2])
                o02 = _nn(zt[0], v02)
                o13 = _nn(zt[1], v13)
                for rr in range(WS):
                    os_[0, pl.ds(off + WP * rr, 8), :] = o02[8 * rr:8 * rr + 8]
                    os_[1, pl.ds(off + WP * rr, 8), :] = o13[8 * rr:8 * rr + 8]
            deps = [(("TR", w), LAG_TR)]
            if w:
                deps.append((("PV", w - 1), 0))
            add(("PV", w), f_pv, deps, mxu=32, valu=3, prio=0)

        for tc in range(WP // ZCH):
            wlast = min((tc * ZCH + ZCH - 1) // WS, NWIN - 1)
            for r in range(WS):
                def f(r=r, tc=tc):
                    trow = pl.ds(r * WP + tc * ZCH, ZCH)
                    o02 = os_[0, trow, :].astype(BF16)
                    o13 = os_[1, trow, :].astype(BF16)
                    acc = (_nt(pltpu.bitcast(woT[0], BF16), o02)
                           + _nt(pltpu.bitcast(woT[1], BF16), o13))
                    cols = pl.ds(tc * ZCH, ZCH)
                    o_ref[r, :, cols] = (x0s[prv, r, :, cols] + acc).astype(BF16)
                add(("Z", r, tc), f, [(("PV", wlast), 150)], mxu=ZCH * 3 // 4, valu=ZCH * 21 // 128, prio=3)

        _emit(tasks)

    for par in range(2):
        pl.when(s % 2 == par)(functools.partial(step, par))


def _emit(tasks):
    T = float(sum(t["mxu"] for t in tasks))
    row = T / WS
    nq = WP // TCH
    qk = lambda w: ATT_BEG + w * (ATT_END * T - ATT_BEG) / NWIN
    pv = lambda w: qk(w) + LAG_QK + TR_LAG + LAG_TR
    zlast = lambda tc: min((tc * ZCH + ZCH - 1) // WS, NWIN - 1)
    for t in tasks:
        n = t["name"]
        k = n[0]
        if k == "Q":
            tau = ((n[1] + 1) * nq + n[2]) * row / nq + Q_SHIFT
        elif k == "U":
            tau = (n[1] - 1) * row - U_AHEAD * row + n[2] * 30
        elif k == "C":
            tau = (n[1] + C_OFF + C_LEN * n[2] / (C // 8)) * row
        elif k == "M":
            tau = (n[1] + C_OFF + C_LEN + 0.01) * row
        elif k == "V":
            tau = (n[1] + C_OFF + C_LEN + 0.02 + 0.08 * n[2] / 12) * row
        elif k == "R":
            tau = (n[1] + C_OFF + C_LEN + 0.11) * row
        elif k == "N":
            tau = (n[1] + C_OFF + C_LEN + 0.13 + 0.1 * n[2] / 12) * row
        elif k == "QK":
            tau = qk(n[1])
        elif k == "SM":
            tau = qk(n[1]) + LAG_QK + n[2]
        elif k == "TR":
            tau = qk(n[1]) + LAG_QK + TR_LAG
        elif k == "PV":
            tau = pv(n[1])
        elif k == "Z":
            beg = pv(zlast(n[2])) + 150
            end = pv(zlast(n[2] + 1)) + 150 if (n[2] + 1) * ZCH < WP else T - 100
            tau = beg + n[1] * (end - beg) / WS
        t["tau"] = tau
    done = {}
    pending = sorted(tasks, key=lambda t: t["tau"])
    now = 0.0
    while pending:
        pick, soonest = None, None
        for t in pending:
            if all(d in done for d, _ in t["deps"]):
                t_ok = max([done[d] + lag for d, lag in t["deps"]], default=0.0)
                if not t["mxu"]:
                    t_ok = max(t_ok, t["tau"] - V_EARLY)
                if t_ok <= now:
                    pick = t
                    break
                soonest = t_ok if soonest is None else min(soonest, t_ok)
        if pick is None:
            now = soonest
            continue
        pending.remove(pick)
        pick["fn"]()
        now += pick["mxu"]
        done[pick["name"]] = now


@jax.jit
def pallas_standalone__window_attn_davit__vision_kernel(
    x: jax.Array,
    dw_pe: jax.Array,
    w_qkv: jax.Array,
    w_o: jax.Array,
):
    B, H, W, Cc = x.shape
    xt = x.reshape(H, W, Cc).transpose(0, 2, 1)
    dwb = jnp.broadcast_to(dw_pe.reshape(9, Cc, 1), (9, Cc, 128)).astype(F32)

    out = pl.pallas_call(
        _kernel,
        grid=(NWIN + 1,),
        in_specs=[
            pl.BlockSpec((WS, Cc, WP), lambda s: (jnp.minimum(s, NWIN - 1), 0, 0)),
            pl.BlockSpec((1, Cc, WP), lambda s: (jnp.minimum(WS * s + WS, H - 1), 0, 0)),
            pl.BlockSpec((9, Cc, 128), lambda s: (0, 0, 0)),
            pl.BlockSpec((Cc, 3 * Cc), lambda s: (0, 0)),
            pl.BlockSpec((Cc, Cc), lambda s: (0, 0)),
        ],
        out_specs=pl.BlockSpec((WS, Cc, WP), lambda s: (jnp.maximum(s - 1, 0), 0, 0)),
        out_shape=jax.ShapeDtypeStruct((H, Cc, W), x.dtype),
        scratch_shapes=[
            pltpu.VMEM((RING, Cc, WP), F32),
            pltpu.VMEM((2, WS, Cc, WP), F32),
            pltpu.VMEM((WS, Cc // 2, WP), U32),
            pltpu.VMEM((2, 6, WS * WP + 8, 128), F32),
            pltpu.VMEM((2, WS * WP + 8, 128), F32),
            pltpu.VMEM((Cc // 2, 640), U32),
            pltpu.VMEM((2, Cc // 2, 128), U32),
            pltpu.VMEM((NS, 2, 56, 128), F32),
            pltpu.VMEM((NS, 64, 128), U32),
        ],
        compiler_params=pltpu.CompilerParams(
            dimension_semantics=("arbitrary",),
            vmem_limit_bytes=100 * 1024 * 1024,
            flags={k: True for k in KFLAGS.split(',') if k} or None,
        ),
    )(xt, xt, dwb, w_qkv, w_o)
    return out.transpose(0, 2, 1).reshape(B, H, W, Cc)
```

```python
import functools
import math

import jax
import jax.numpy as jnp
from jax import lax
import jax.experimental.pallas as pl
import jax.experimental.pallas.tpu as pltpu

F32 = jnp.float32
BF16 = jnp.bfloat16
U32 = jnp.uint32

WS = 7
NH = 4
C = 192
DH = C // NH
HH = 511
WP = 512
NWIN = HH // WS
RING = 14
CCH = 8
TCH = 128
ZCH = 128
INFLIGHT = 8
LAG_QK = 120
LAG_TR = 200
ATT_BEG = 300.0
ATT_END = 0.85
Q_SHIFT = 0.0
U_AHEAD = 0.3
C_OFF = -0.1
C_LEN = 0.6
V_EARLY = 100.0
NS = 16
STAGE_S = 1
STAGE_Z = 1
TR_LAG = 60
KFLAGS = 'XLA_TPU_EVENLY_DISTRIBUTE_CRITICAL_NODES'


def _nt(a, b):
    return lax.dot_general(a, b, (((1,), (1,)), ((), ())), preferred_element_type=F32)


def _nn(a, b):
    return lax.dot_general(a, b, (((1,), (0,)), ((), ())), preferred_element_type=F32)


def _tn(a, b):
    return lax.dot_general(a, b, (((0,), (0,)), ((), ())), preferred_element_type=F32)


def _pack2(lo, hi):
    u = pltpu.pack_elementwise([lo, hi], packed_dtype=BF16)
    return u if u.dtype == U32 else pltpu.bitcast(u, U32)


def _pack_rows(t):
    t = t.astype(F32)
    return jnp.concatenate(
        [_pack2(t[16 * g:16 * g + 8], t[16 * g + 8:16 * g + 16]) for g in range(t.shape[0] // 16)], axis=0)


def _sub_reduce(x, op):
    x = op(x, pltpu.roll(x, 4, 0))
    x = op(x, pltpu.roll(x, 2, 0))
    x = op(x, pltpu.roll(x, 1, 0))
    return x


def _kernel(xm_ref, xn_ref, dw_ref, wqkv_ref, wo_ref, o_ref,
            xs, x0s, hts, qkv, os_, w640, woT, s_scr, z_scr):
    s = pl.program_id(0)
    nsteps = pl.num_programs(0)

    lane = lax.broadcasted_iota(jnp.int32, (1, 128), 1)

    @pl.when(s == 0)
    def _prep():
        wq = wqkv_ref[:, 0:C].astype(F32) * (DH ** -0.5 * math.log2(math.e))
        wq = wq.astype(BF16)
        wk = wqkv_ref[:, C:2 * C]
        wv = wqkv_ref[:, 2 * C:3 * C]
        z32 = jnp.zeros((C, 32), BF16)
        v13 = jnp.concatenate([wv[:, DH:2 * DH], wv[:, 3 * DH:4 * DH]], axis=1)
        t0 = jnp.concatenate([v13[:, 0:32], wq[:, 0:96]], axis=1)
        t1 = jnp.concatenate([z32, wk[:, 0:96]], axis=1)
        t2 = jnp.concatenate([wq[:, 96:128], v13[:, 32:64], wq[:, 128:192]], axis=1)
        t3 = jnp.concatenate([wk[:, 96:128], z32, wk[:, 128:192]], axis=1)
        t4 = jnp.concatenate([wv[:, 0:DH], wv[:, 2 * DH:3 * DH], v13[:, 64:96]], axis=1)
        w640[:, 0:128] = _pack_rows(t0)
        w640[:, 128:256] = _pack_rows(t1)
        w640[:, 256:384] = _pack_rows(t2)
        w640[:, 384:512] = _pack_rows(t3)
        w640[:, 512:640] = _pack_rows(t4)
        wo = wo_ref[...]
        zr = jnp.zeros((32, C), BF16)
        r02 = jnp.concatenate([wo[0:DH], wo[2 * DH:3 * DH], zr], axis=0)
        r13 = jnp.concatenate([wo[DH:2 * DH], wo[3 * DH:3 * DH + 16], zr,
                               wo[3 * DH + 16:4 * DH]], axis=0)
        woT[0] = pltpu.bitcast(r02.astype(F32).T.astype(BF16), U32)
        woT[1] = pltpu.bitcast(r13.astype(F32).T.astype(BF16), U32)
        xs[RING - 1] = jnp.zeros((C, WP), F32)
        hts[WS - 1] = jnp.zeros((C // 2, WP), U32)
        x0s[1] = jnp.zeros((WS, C, WP), F32)

        def zbody(i, c):
            rows = pl.ds(pl.multiple_of(i * 8, 8), 8)
            for t in range(6):
                qkv[1, t, rows, :] = jnp.zeros((8, 128), F32)
            return c
        lax.fori_loop(0, WS * WP // 8 + 1, zbody, 0)
        for t in range(6):
            qkv[0, t, pl.ds(WS * WP, 8), :] = jnp.zeros((8, 128), F32)

    wmask = lax.broadcasted_iota(jnp.int32, (1, WP), 1) < HH
    last = nsteps - 2

    def put_rows(slot, rows, src, valid=None):
        v = src.astype(F32)
        m = wmask if valid is None else jnp.logical_and(wmask, valid)
        xs[slot, rows, :] = jnp.where(m, v, 0.0)

    @pl.when(s == 0)
    def _():
        put_rows(0, pl.ds(0, C), xm_ref[0])

    def step(cur):
        prv = 1 - cur
        g0 = WS * cur
        tasks = []

        def add(name, fn, deps=(), mxu=0, valu=0, prio=0):
            tasks.append(dict(name=name, fn=fn, deps=list(deps), mxu=mxu, valu=valu, prio=prio))

        UCH = 48
        for k in range(1, WS + 1):
            for ui in range(C // UCH):
                def f(k=k, ui=ui):
                    rows = pl.ds(ui * UCH, UCH)
                    if k < WS:
                        put_rows((g0 + k) % RING, rows, xm_ref[k, rows, :])
                    else:
                        put_rows((g0 + k) % RING, rows, xn_ref[0, rows, :], s < last)
                add(("U", k, ui), f, valu=28, prio=(k - 1) * 100 + ui)

        st = {}
        CH = CCH
        NCI = C // CH
        for r in range(WS):
            for ci in range(NCI):
                def f(r=r, ci=ci):
                    rows = pl.ds(ci * CH, CH)
                    top = xs[(g0 + r + RING - 1) % RING, rows, :]
                    mid = xs[(g0 + r) % RING, rows, :]
                    bot = xs[(g0 + r + 1) % RING, rows, :]

                    def coef(i, j):
                        cf = dw_ref[i * 3 + j, rows, :]
                        return jnp.concatenate([cf] * (WP // 128), axis=1)

                    t0 = top * coef(0, 0) + mid * coef(1, 0) + bot * coef(2, 0)
                    t1 = top * coef(0, 1) + mid * coef(1, 1) + bot * coef(2, 1)
                    t2 = top * coef(0, 2) + mid * coef(1, 2) + bot * coef(2, 2)
                    x0 = mid + (pltpu.roll(t0, 1, 1) + t1 + pltpu.roll(t2, WP - 1, 1))
                    x0s[cur, r, rows, :] = x0
                    part = x0[0:8]
                    for k in range(1, CH // 8):
                        part = part + x0[8 * k:8 * k + 8]
                    st[("s", r)] = part if ci == 0 else st[("s", r)] + part
                deps = [(("U", r + 1, ci * CH // UCH), 40)]
                if ci:
                    deps.append((("C", r, ci - 1), 0))
                add(("C", r, ci), f, deps, valu=3 * CH, prio=r * 100 + 10 + ci)

            def f(r=r):
                st[("m", r)] = _sub_reduce(st.pop(("s", r)), jnp.add) * (1.0 / C)
            add(("M", r), f, [(("C", r, NCI - 1), 0)], valu=8, prio=r * 100 + 40)

            for ci in range(C // 16):
                def f(r=r, ci=ci):
                    mean = st[("m", r)]
                    acc = None
                    for hf in range(2):
                        d = x0s[cur, r, pl.ds(ci * 16 + hf * 8, 8), :] - mean
                        acc = d * d if acc is None else acc + d * d
                    st[("v", r)] = acc if ci == 0 else st[("v", r)] + acc
                deps = [(("M", r), 10)] if ci == 0 else [(("V", r, ci - 1), 0)]
                add(("V", r, ci), f, deps, valu=6, prio=r * 100 + 50 + ci)

            def f(r=r):
                var = _sub_reduce(st.pop(("v", r)), jnp.add) * (1.0 / C)
                st[("r", r)] = lax.rsqrt(var + 1e-5)
                st[("o", r)] = -st[("m", r)] * st[("r", r)]
            add(("R", r), f, [(("V", r, C // 16 - 1), 0)], valu=10, prio=r * 100 + 70)

            for ci in range(C // 16):
                def f(r=r, ci=ci):
                    rstd = st[("r", r)]
                    shift = st[("o", r)]
                    lo = x0s[cur, r, pl.ds(ci * 16, 8), :] * rstd + shift
                    hi = x0s[cur, r, pl.ds(ci * 16 + 8, 8), :] * rstd + shift
                    hts[r, pl.ds(ci * 8, 8), :] = _pack2(lo, hi)
                deps = [(("R", r), 30)]
                if r == WS - 1:
                    deps.append((("Q", -1, WP // TCH - 1), 0))
                add(("N", r, ci), f, deps, valu=6, prio=r * 100 + 80 + ci)

        for r in range(-1, WS - 1):
            for tc in range(WP // TCH):
                def f(r=r, tc=tc):
                    rr = r % WS
                    slot = prv if r < 0 else cur
                    ht = pltpu.bitcast(hts[rr, :, tc * TCH:(tc + 1) * TCH], BF16)
                    res = _tn(ht, pltpu.bitcast(w640[...], BF16))
                    trow = pl.ds(rr * WP + tc * TCH, TCH)
                    t0 = res[:, 0:128]
                    t2 = res[:, 256:384]
                    t4 = res[:, 512:640]
                    qkv[slot, 0, trow, :] = t0
                    qkv[slot, 1, trow, :] = res[:, 128:256]
                    qkv[slot, 2, trow, :] = t2
                    qkv[slot, 3, trow, :] = res[:, 384:512]
                    qkv[slot, 4, trow, :] = t4
                    qkv[slot, 5, trow, :] = jnp.where(lane < 32, t0, jnp.where(lane < 64, t2, t4))
                deps = []
                if r >= 0:
                    deps.append((("N", r, C // 16 - 1), 60))
                if tc:
                    deps.append((("Q", r, tc - 1), 0))
                elif r >= 0:
                    deps.append((("Q", r - 1, WP // TCH - 1), 0))
                add(("Q", r, tc), f, deps, mxu=TCH * 10 // 4, valu=TCH * 112 // 128 // 4, prio=2)

        sub = lax.broadcasted_iota(jnp.int32, (8, 128), 0)
        key_ok = sub < WS
        ln = lax.broadcasted_iota(jnp.int32, (8, 128), 1)
        mq = [
            jnp.logical_and(ln >= 32, ln < 80),
            ln >= 80,
            jnp.logical_or(ln < 32, jnp.logical_and(ln >= 64, ln < 80)),
            ln >= 80,
        ]
        ones = jnp.full((8, 128), 0xFFFFFFFF, U32)
        zeros = jnp.zeros((8, 128), U32)
        mv = [
            jnp.where(ln < 48, ones, zeros),
            jnp.where(jnp.logical_and(ln >= 48, ln < 96), ones, zeros),
            jnp.where(jnp.logical_or(jnp.logical_and(ln >= 48, ln < 64), ln >= 96), ones, zeros),
        ]
        zero8 = jnp.zeros((8, 128), F32)

        def load56(t, off):
            return [qkv[prv, t, pl.ds(off + WP * rr, 8), :] for rr in range(WS)]

        def pack64(parts):
            pz = parts + [zero8]
            return [_pack2(pz[2 * i], pz[2 * i + 1]) for i in range(4)]

        def bd(parts, ma, mb):
            za = [jnp.where(ma, v, 0.0) for v in parts] + [zero8]
            zb = [jnp.where(mb, v, 0.0) for v in parts] + [zero8]
            return jnp.concatenate(za + zb, axis=0).astype(BF16)

        def bdv(parts, ma, mb):
            us = pack64(parts)
            return pltpu.bitcast(jnp.concatenate([u & ma for u in us] + [u & mb for u in us], axis=0), BF16)

        def softmax_t(stv):
            parts = [stv[8 * i:8 * i + 8] for i in range(WS)]
            m = parts[0]
            for p in parts[1:]:
                m = jnp.maximum(m, p)
            m = jnp.where(key_ok, m, -jnp.inf)
            m = _sub_reduce(m, jnp.maximum)
            m = jnp.where(key_ok, m, jnp.inf)
            es = [jnp.exp2(p - m) for p in parts]
            l = es[0]
            for e in es[1:]:
                l = l + e
            l = _sub_reduce(l, jnp.add)
            rcp = pl.reciprocal(l, approx=True)
            rcp = rcp * (2.0 - l * rcp)
            return pack64([e * rcp for e in es])

        for w in range(NWIN):
            off = WS * w
            tcw = min((off + 7) // TCH, WP // TCH - 1)

            def f_qk(w=w, off=off):
                k01 = jnp.concatenate(load56(1, off), axis=0)
                k23 = jnp.concatenate(load56(3, off), axis=0)
                q01 = bd(load56(0, off), mq[0], mq[1])
                q23 = bd(load56(2, off), mq[2], mq[3])
                if STAGE_S:
                    s_scr[w % NS, 0] = _nt(k01, q01)
                    s_scr[w % NS, 1] = _nt(k23, q23)
                else:
                    st[("S", w)] = (_nt(k01, q01), _nt(k23, q23))
            deps = [(("Q", -1, tcw), 200)]
            if w:
                deps.append((("QK", w - 1), 0))
            if w >= INFLIGHT:
                deps.append((("PV", w - INFLIGHT), 0))
            add(("QK", w), f_qk, deps, mxu=28, valu=5, prio=1)

            for hp in range(2):
                def f_sm(w=w, hp=hp):
                    if STAGE_S:
                        st[("P", w, hp)] = softmax_t(s_scr[w % NS, hp])
                    else:
                        st[("P", w, hp)] = softmax_t(st[("S", w)][hp])
                        if hp == 1:
                            del st[("S", w)]
                add(("SM", w, hp), f_sm, [(("QK", w), LAG_QK)] + ([(("SM", w, 0), 0)] if hp else []),
                    valu=14, prio=-1)

            def f_tr(w=w):
                z = pltpu.bitcast(jnp.concatenate(st.pop(("P", w, 0)) + st.pop(("P", w, 1)), axis=0), BF16)
                zt = z.T
                if STAGE_Z:
                    z_scr[w % NS] = pltpu.bitcast(zt, U32)
                else:
                    st[("Z", w)] = (zt[0:64], zt[64:128])
            add(("TR", w), f_tr, [(("SM", w, 1), 20)], valu=6, prio=-2)

            def f_pv(w=w, off=off):
                if STAGE_Z:
                    zt = (pltpu.bitcast(z_scr[w % NS, 0:32], BF16),
                          pltpu.bitcast(z_scr[w % NS, 32:64], BF16))
                else:
                    zt = st.pop(("Z", w))
                v02 = bdv(load56(4, off), mv[0], mv[1])
                v13 = bdv(load56(5, off), mv[0], mv[2])
                o02 = _nn(zt[0], v02)
                o13 = _nn(zt[1], v13)
                for rr in range(WS):
                    os_[0, pl.ds(off + WP * rr, 8), :] = o02[8 * rr:8 * rr + 8]
                    os_[1, pl.ds(off + WP * rr, 8), :] = o13[8 * rr:8 * rr + 8]
            deps = [(("TR", w), LAG_TR)]
            if w:
                deps.append((("PV", w - 1), 0))
            add(("PV", w), f_pv, deps, mxu=32, valu=3, prio=0)

        for tc in range(WP // ZCH):
            wlast = min((tc * ZCH + ZCH - 1) // WS, NWIN - 1)
            for r in range(WS):
                def f(r=r, tc=tc):
                    trow = pl.ds(r * WP + tc * ZCH, ZCH)
                    o02 = os_[0, trow, :].astype(BF16)
                    o13 = os_[1, trow, :].astype(BF16)
                    acc = (_nt(pltpu.bitcast(woT[0], BF16), o02)
                           + _nt(pltpu.bitcast(woT[1], BF16), o13))
                    cols = pl.ds(tc * ZCH, ZCH)
                    o_ref[r, :, cols] = (x0s[prv, r, :, cols] + acc).astype(BF16)
                add(("Z", r, tc), f, [(("PV", wlast), 150)], mxu=ZCH * 3 // 4, valu=ZCH * 21 // 128, prio=3)

        _emit(tasks)

    for par in range(2):
        pl.when(s % 2 == par)(functools.partial(step, par))


def _emit(tasks):
    T = float(sum(t["mxu"] for t in tasks))
    row = T / WS
    nq = WP // TCH
    qk = lambda w: ATT_BEG + w * (ATT_END * T - ATT_BEG) / NWIN
    pv = lambda w: qk(w) + LAG_QK + TR_LAG + LAG_TR
    zlast = lambda tc: min((tc * ZCH + ZCH - 1) // WS, NWIN - 1)
    for t in tasks:
        n = t["name"]
        k = n[0]
        if k == "Q":
            tau = ((n[1] + 1) * nq + n[2]) * row / nq + Q_SHIFT
        elif k == "U":
            tau = (n[1] - 1) * row - U_AHEAD * row + n[2] * 30
        elif k == "C":
            tau = (n[1] + C_OFF + C_LEN * n[2] / (C // CCH)) * row
        elif k == "M":
            tau = (n[1] + C_OFF + C_LEN + 0.01) * row
        elif k == "V":
            tau = (n[1] + C_OFF + C_LEN + 0.02 + 0.08 * n[2] / 12) * row
        elif k == "R":
            tau = (n[1] + C_OFF + C_LEN + 0.11) * row
        elif k == "N":
            tau = (n[1] + C_OFF + C_LEN + 0.13 + 0.1 * n[2] / 12) * row
        elif k == "QK":
            tau = qk(n[1])
        elif k == "SM":
            tau = qk(n[1]) + LAG_QK + n[2]
        elif k == "TR":
            tau = qk(n[1]) + LAG_QK + TR_LAG
        elif k == "PV":
            tau = pv(n[1])
        elif k == "Z":
            beg = pv(zlast(n[2])) + 150
            end = pv(zlast(n[2] + 1)) + 150 if (n[2] + 1) * ZCH < WP else T - 100
            tau = beg + n[1] * (end - beg) / WS
        t["tau"] = tau
    done = {}
    pending = sorted(tasks, key=lambda t: t["tau"])
    now = 0.0
    while pending:
        pick, soonest = None, None
        for t in pending:
            if all(d in done for d, _ in t["deps"]):
                t_ok = max([done[d] + lag for d, lag in t["deps"]], default=0.0)
                if not t["mxu"]:
                    t_ok = max(t_ok, t["tau"] - V_EARLY)
                if t_ok <= now:
                    pick = t
                    break
                soonest = t_ok if soonest is None else min(soonest, t_ok)
        if pick is None:
            now = soonest
            continue
        pending.remove(pick)
        pick["fn"]()
        now += pick["mxu"]
        done[pick["name"]] = now


@jax.jit
def pallas_standalone__window_attn_davit__vision_kernel(
    x: jax.Array,
    dw_pe: jax.Array,
    w_qkv: jax.Array,
    w_o: jax.Array,
):
    B, H, W, Cc = x.shape
    xt = x.reshape(H, W, Cc).transpose(0, 2, 1)
    dwb = jnp.broadcast_to(dw_pe.reshape(9, Cc, 1), (9, Cc, 128)).astype(F32)

    out = pl.pallas_call(
        _kernel,
        grid=(NWIN + 1,),
        in_specs=[
            pl.BlockSpec((WS, Cc, WP), lambda s: (jnp.minimum(s, NWIN - 1), 0, 0)),
            pl.BlockSpec((1, Cc, WP), lambda s: (jnp.minimum(WS * s + WS, H - 1), 0, 0)),
            pl.BlockSpec((9, Cc, 128), lambda s: (0, 0, 0)),
            pl.BlockSpec((Cc, 3 * Cc), lambda s: (0, 0)),
            pl.BlockSpec((Cc, Cc), lambda s: (0, 0)),
        ],
        out_specs=pl.BlockSpec((WS, Cc, WP), lambda s: (jnp.maximum(s - 1, 0), 0, 0)),
        out_shape=jax.ShapeDtypeStruct((H, Cc, W), x.dtype),
        scratch_shapes=[
            pltpu.VMEM((RING, Cc, WP), F32),
            pltpu.VMEM((2, WS, Cc, WP), F32),
            pltpu.VMEM((WS, Cc // 2, WP), U32),
            pltpu.VMEM((2, 6, WS * WP + 8, 128), F32),
            pltpu.VMEM((2, WS * WP + 8, 128), F32),
            pltpu.VMEM((Cc // 2, 640), U32),
            pltpu.VMEM((2, Cc // 2, 128), U32),
            pltpu.VMEM((NS, 2, 56, 128), F32),
            pltpu.VMEM((NS, 64, 128), U32),
        ],
        compiler_params=pltpu.CompilerParams(
            dimension_semantics=("arbitrary",),
            vmem_limit_bytes=100 * 1024 * 1024,
            flags={k: True for k in KFLAGS.split(',') if k} or None,
        ),
    )(xt, xt, dwb, w_qkv, w_o)
    return out.transpose(0, 2, 1).reshape(B, H, W, Cc)
```
